```python
import os as _os
_os.environ.setdefault("JAX_PLATFORMS", "cpu")
import jax
import jax.numpy as jnp

def _softmax(x, axis=-1):
    return jax.nn.softmax(x, axis=axis)
def _gelu(x):
    return jax.nn.gelu(x, approximate=True)
def _silu(x):
    return jax.nn.silu(x)
def _sigmoid(x):
    return jax.nn.sigmoid(x)
def _layernorm(x, axis=-1, eps=1e-5):
    m = jnp.mean(x, axis=axis, keepdims=True)
    v = jnp.var(x, axis=axis, keepdims=True)
    return (x - m) / jnp.sqrt(v + eps)
def _scatter_add(tgt, idx, src, axis=0):
    return tgt.at[idx].add(src)
def _segment_sum(src, seg, n):
    return jax.ops.segment_sum(src, seg, n)
class _Rng:
    def __init__(self, key):
        self._k = key
    def _next(self):
        self._k, sub = jax.random.split(self._k)
        return sub
    def normal(self, shape):
        return jax.random.normal(self._next(), shape, dtype=jnp.bfloat16)
    def randint(self, lo, hi, shape):
        return jax.random.randint(self._next(), shape, lo, hi, dtype=jnp.int32)
    def uniform(self, shape, lo=0.0, hi=1.0):
        return jax.random.uniform(self._next(), shape, jnp.bfloat16, lo, hi)
    def permutation(self, n):
        return jax.random.permutation(self._next(), n)


kernel_name = 'concat_heads__mha_block_cached__mha_block_cached__near_ridge'

def setup_inputs():
    _rng = _Rng(jax.random.key(int.from_bytes(__import__("os").urandom(4), "little")))
    _w = (lambda a: (lambda t: t.astype(jnp.bfloat16) if jnp.issubdtype(t.dtype, jnp.floating) else t)(jnp.asarray(a)))
    def _A_setup():
        B, Sq, D = 8, 144, 640
        H, Sk, Dh = 32, 512, 128
        return {
            "x": _w((lambda *s: _rng.normal(s) * 0.8)(B, Sq, D)),
            "k_cache": _w((lambda *s: _rng.normal(s) * 0.8)(B, H, Sk, Dh)),
            "v_cache": _w((lambda *s: _rng.normal(s) * 0.05)(B, H, Sk, Dh)),
            "wq": _w((lambda *s: _rng.normal(s) * 0.8)(D, H * Dh) * (D ** -0.5)),
            "wo": _w((lambda *s: _rng.normal(s) * 0.05)(H * Dh, D) * ((H * Dh) ** -0.5)),
        }
    _A_in = _A_setup()

    def _B_setup():
        B, Sq, D = 8, 144, 640
        H, Sk, Dh = 32, 512, 128
        return {
            "x": _w((lambda *s: _rng.normal(s) * 0.8)(B, Sq, D)),
            "k_cache": _w((lambda *s: _rng.normal(s) * 0.8)(B, H, Sk, Dh)),
            "v_cache": _w((lambda *s: _rng.normal(s) * 0.05)(B, H, Sk, Dh)),
            "wq": _w((lambda *s: _rng.normal(s) * 0.8)(D, H * Dh) * (D ** -0.5)),
            "wo": _w((lambda *s: _rng.normal(s) * 0.05)(H * Dh, D) * ((H * Dh) ** -0.5)),
        }
    _B_in = _B_setup()

    return {
        "A_x": _A_in["x"],
        "A_k_cache": _A_in["k_cache"],
        "A_v_cache": _A_in["v_cache"],
        "A_wq": _A_in["wq"],
        "A_wo": _A_in["wo"],
        "B_x": _B_in["x"],
        "B_k_cache": _B_in["k_cache"],
        "B_v_cache": _B_in["v_cache"],
        "B_wq": _B_in["wq"],
        "B_wo": _B_in["wo"],
    }

def reference(A_x, A_k_cache, A_v_cache, A_wq, A_wo, B_x, B_k_cache, B_v_cache, B_wq, B_wo):
    def _A_ref(x, k_cache, v_cache, wq, wo):
        B, Sq, D = x.shape
        H, Dh = 32, 128
        q = (lambda x, *d: x.transpose(*d))((x @ wq).reshape(B, Sq, H, Dh), 0, 2, 1, 3)
        scores = jnp.einsum("bhqd,bhkd->bhqk", q, k_cache) * (Dh ** -0.5)
        p = _softmax(scores, axis=-1)
        o = jnp.einsum("bhqk,bhkd->bhqd", p, v_cache)
        return (lambda x, *d: x.transpose(*d))(o, 0, 2, 1, 3).reshape(B, Sq, H * Dh) @ wo

    def _B_ref(x, k_cache, v_cache, wq, wo):
        B, Sq, D = x.shape
        H, Dh = 32, 128
        q = (lambda x, *d: x.transpose(*d))((x @ wq).reshape(B, Sq, H, Dh), 0, 2, 1, 3)
        scores = jnp.einsum("bhqd,bhkd->bhqk", q, k_cache) * (Dh ** -0.5)
        p = _softmax(scores, axis=-1)
        o = jnp.einsum("bhqk,bhkd->bhqd", p, v_cache)
        return (lambda x, *d: x.transpose(*d))(o, 0, 2, 1, 3).reshape(B, Sq, H * Dh) @ wo

    a = _A_ref(A_x, A_k_cache, A_v_cache, A_wq, A_wo)
    b = _B_ref(B_x, B_k_cache, B_v_cache, B_wq, B_wo)
    return jnp.concatenate([a, b], axis=-1)
```

```python
import math, functools
import jax, jax.numpy as jnp
from jax import lax
import jax.experimental.pallas as pl
import jax.experimental.pallas.tpu as pltpu

B, Sq, D = 8, 144, 640
H, Sk, Dh = 32, 512, 128
M = B * Sq
NC = D // 128
QSCALE = (Dh ** -0.5) * math.log2(math.e)

def gen_order(G, pat, olag=3, plag=1, dpos=1):
    n_units = G * B
    toks = []
    for n in range(n_units + max(olag, plag)):
        for k in pat:
            if k == "S" and n < n_units: toks.append(("S", n))
            if k == "Q" and n < n_units: toks.append(("Q", n))
            if k == "P" and 0 <= n - plag < n_units: toks.append(("P", n - plag))
            if k == "O" and 0 <= n - olag < n_units: toks.append(("O", n - olag))
        if n < n_units and n % B == dpos: toks.append(("D", n // B))
    return toks

def make(G=1, nd=None, pat="SOQP", olag=3, plag=1, dpos=1, flags=None, order=None, dbc=True, waittop=True, dtop=False):
    NI = 2 * H // G
    NIB = H // G
    ND = nd or {1: 4, 2: 3, 4: 2}[G] ;
    if G == 4 and nd is None: ND = 3
    toks = gen_order(G, pat, olag, plag, dpos) if order is None else [(t[0], int(t[1:])) for t in order.split()]

    def ld(ref):
        return pltpu.bitcast(ref.bitcast(jnp.uint32)[...], jnp.bfloat16)

    def kern(ax, ak, av, awq, awo, bx, bk, bv, bwq, bwo, out,
             xs, kb, vb, wqb, wob, qb, acc, stage, ksem, vsem, osem_, qsem, xsem, osem):
        srcs = ((ax, ak, av, awq, awo), (bx, bk, bv, bwq, bwo))

        def k_copy(br, h, slot, u): return pltpu.make_async_copy(srcs[br][1].at[:, h], kb.at[slot, u], ksem.at[slot, u])
        def v_copy(br, h, slot, u): return pltpu.make_async_copy(srcs[br][2].at[:, h], vb.at[slot, u], vsem.at[slot, u])
        def wo_copies(br, h, slot, u):
            return [pltpu.make_async_copy(srcs[br][4].at[pl.ds(pl.multiple_of(h * Dh, Dh), Dh), pl.ds(c * 128, 128)],
                                          wob.at[slot, u, c], osem_.at[slot, u]) for c in range(NC)]
        def wq_copy(br, h, slot, u):
            return pltpu.make_async_copy(srcs[br][3].at[:, pl.ds(pl.multiple_of(h * Dh, Dh), Dh)], wqb.at[slot, u], qsem.at[slot, u])
        def x_copies(br):
            return [pltpu.make_async_copy(srcs[br][0].at[:, pl.ds(c * 128, 128)], xs.at[br, c], xsem.at[br]) for c in range(NC)]
        def out_copy(br):
            return pltpu.make_async_copy(stage.at[br], out.at[:, pl.ds(br * D, D)], osem.at[br])

        def start_head(t, slot, u):
            @pl.when(t < H)
            def _():
                k_copy(0, t, slot, u).start(); v_copy(0, t, slot, u).start()
                for c in wo_copies(0, t, slot, u): c.start()
            @pl.when(jnp.logical_and(t >= H, t < 2 * H))
            def _():
                k_copy(1, t - H, slot, u).start(); v_copy(1, t - H, slot, u).start()
                for c in wo_copies(1, t - H, slot, u): c.start()
            @pl.when(t + 1 < H)
            def _():
                wq_copy(0, t + 1, slot, u).start()
            @pl.when(jnp.logical_and(t + 1 >= H, t < 2 * H))
            def _():
                wq_copy(1, jnp.minimum(t + 1 - H, H - 1), slot, u).start()

        def qproj(br, par, wq_ref, b):
            rows = pl.ds(b * Sq, Sq)
            r = None
            for c in range(NC):
                d = jnp.dot(ld(xs.at[br, c, rows]), ld(wq_ref.at[pl.ds(c * 128, 128)]), preferred_element_type=jnp.float32)
                r = d if r is None else r + d
            qb[par, rows, :] = (r * QSCALE).astype(jnp.bfloat16)

        for c in x_copies(0): c.start()
        wq_copy(0, 0, ND - 1, G - 1).start()
        def pro(j, c):
            for u in range(G):
                start_head(j * G + u, j, u)
            return c
        lax.fori_loop(0, ND - 1, pro, None)
        acc[...] = jnp.zeros_like(acc)
        for c in x_copies(0): c.wait()
        wq_copy(0, 0, ND - 1, G - 1).wait()
        for b in range(B):
            qproj(0, 0, wqb.at[ND - 1, G - 1], b)

        def body(i, carry):
            slot = lax.rem(i, ND) if ND & (ND - 1) else i & (ND - 1)
            pslot = jnp.where(slot == 0, ND - 1, slot - 1)
            br = i // NIB if NIB & (NIB - 1) else i >> int(math.log2(NIB))
            cache = {}
            waited = set()
            def wait(kind, u):
                if (kind, u) in waited: return
                waited.add((kind, u))
                if kind == "k": k_copy(0, 0, slot, u).wait()
                if kind == "v": v_copy(0, 0, slot, u).wait()
                if kind == "q": wq_copy(0, 0, slot, u).wait()
                if kind == "o":
                    for c in wo_copies(0, 0, slot, u): c.wait()

            def S(n):
                u, b = divmod(n, B)
                wait("k", u)
                par = (u & 1) if G % 2 == 0 else (i * G + u) & 1
                q = ld(qb.at[par, pl.ds(b * Sq, Sq)])
                k = ld(kb.at[slot, u, b])
                sc = lax.dot_general(q, k, (((1,), (1,)), ((), ())), preferred_element_type=jnp.float32)
                m = jnp.max(sc, axis=-1, keepdims=True)
                p = jnp.exp2(sc - m)
                l = jnp.sum(p, axis=-1, keepdims=True)
                r0 = pl.reciprocal(l, approx=True)
                rl = r0 * (2.0 - l * r0)
                return p.astype(jnp.bfloat16), rl

            def P(n, p, rl):
                u, b = divmod(n, B)
                wait("v", u)
                o = jnp.dot(p, ld(vb.at[slot, u, b]), preferred_element_type=jnp.float32)
                return (o * rl).astype(jnp.bfloat16)

            def O(n, o):
                u, b = divmod(n, B)
                wait("o", u)
                rows = pl.ds(b * Sq, Sq)
                for c in range(NC):
                    acc[br, rows, c * 128:(c + 1) * 128] += jnp.dot(o, ld(wob.at[slot, u, c]), preferred_element_type=jnp.float32)

            def Q(n):
                u, b = divmod(n, B)
                wait("q", u)
                npar = ((u + 1) & 1) if G % 2 == 0 else (i * G + u + 1) & 1
                if u < G - 1:
                    brn = br
                else:
                    brn = jnp.minimum((i + 1) >> int(math.log2(NIB)), 1)
                qproj(brn, npar, wqb.at[slot, u], b)

            def Dm(u):
                start_head((i + ND - 1) * G + u, pslot, u)

            if dtop:
                for u in range(G): Dm(u)
            if waittop:
                for u in range(G):
                    for kind in "qkvo": wait(kind, u)
            st, ov = {}, {}
            for kind, n in toks:
                if kind == "S": st[n] = S(n)
                elif kind == "P": ov[n] = P(n, *st.pop(n))
                elif kind == "O": O(n, ov.pop(n))
                elif kind == "Q": Q(n)
                elif kind == "D" and not dtop: Dm(n)

            @pl.when(i == NIB - 1)
            def _():
                stage[0] = acc[0].astype(jnp.bfloat16)
                out_copy(0).start()
            @pl.when(i == NIB - 3)
            def _():
                for c in x_copies(1): c.wait()
            @pl.when(i == NIB // 2)
            def _():
                for c in x_copies(1): c.start()
            return carry

        lax.fori_loop(0, NI, body, None)
        stage[1] = acc[1].astype(jnp.bfloat16)
        out_copy(1).start()
        out_copy(0).wait()
        out_copy(1).wait()

    def run(ax, ak, av, awq, awo, bx, bk, bv, bwq, bwo):
        anyspec = pl.BlockSpec(memory_space=pl.ANY)
        out = pl.pallas_call(
            kern,
            in_specs=[anyspec] * 10,
            out_specs=anyspec,
            out_shape=jax.ShapeDtypeStruct((M, 2 * D), jnp.bfloat16),
            scratch_shapes=[
                pltpu.VMEM((2, NC, M, 128), jnp.bfloat16),
                pltpu.VMEM((ND, G, B, Sk, Dh), jnp.bfloat16),
                pltpu.VMEM((ND, G, B, Sk, Dh), jnp.bfloat16),
                pltpu.VMEM((ND, G, D, Dh), jnp.bfloat16),
                pltpu.VMEM((ND, G, NC, Dh, 128), jnp.bfloat16),
                pltpu.VMEM((2, M, Dh), jnp.bfloat16),
                pltpu.VMEM((2, M, D), jnp.float32),
                pltpu.VMEM((2, M, D), jnp.bfloat16),
                pltpu.SemaphoreType.DMA((ND, G)),
                pltpu.SemaphoreType.DMA((ND, G)),
                pltpu.SemaphoreType.DMA((ND, G)),
                pltpu.SemaphoreType.DMA((ND, G)),
                pltpu.SemaphoreType.DMA((2,)),
                pltpu.SemaphoreType.DMA((2,)),
            ],
            compiler_params=pltpu.CompilerParams(vmem_limit_bytes=100*1024*1024, flags=flags, disable_bounds_checks=dbc),
        )(ax.reshape(M, D), ak, av, awq, awo, bx.reshape(M, D), bk, bv, bwq, bwo)
        return out.reshape(B, Sq, 2 * D)
    return run


_run = make(G=2, nd=4, pat="QSPO")


@jax.jit
def pallas_concat_heads__mha_block_cached__mha_block_cached__near_ridge_kernel(
    A_x, A_k_cache, A_v_cache, A_wq, A_wo, B_x, B_k_cache, B_v_cache, B_wq, B_wo
):
    return _run(A_x, A_k_cache, A_v_cache, A_wq, A_wo, B_x, B_k_cache, B_v_cache, B_wq, B_wo)
```

```python
import math

import jax
import jax.numpy as jnp
from jax import lax
import jax.experimental.pallas as pl
import jax.experimental.pallas.tpu as pltpu

B, SQ, D = 8, 144, 640
H, SK, DH = 32, 512, 128
M = B * SQ
NC = D // 128
QSCALE = (DH ** -0.5) * math.log2(math.e)

GQ = 8
NJ = 2 * H // GQ
NJB = H // GQ
NQ = 3
G = 4
NS = 6
N8 = 6
N4 = (2 * H - 8 * N8) // 4
HPJ = 16 // NJ


def _order(heads, dma_after):
    n_units = heads * B
    toks = []
    for n in range(n_units + 2):
        if n < n_units:
            toks.append(("S", n))
        if 0 <= n - 1 < n_units:
            toks.append(("P", n - 1))
        if 0 <= n - 2 < n_units:
            toks.append(("O", n - 2))
        if n in dma_after:
            toks.append(("D", dma_after.index(n)))
    return toks


def _ld(ref):
    return pltpu.bitcast(ref.bitcast(jnp.uint32)[...], jnp.bfloat16)


def _dot(a, b):
    return jnp.dot(a, b, preferred_element_type=jnp.float32)


def _kernel(ax, ak, av, awq, awo, bx, bk, bv, bwq, bwo, out,
            xs, kvb, wqb, wob, qall, acc, stage, kvsem, wosem, qsem, psem, osem):
    srcs = ((ax, ak, av, awq, awo), (bx, bk, bv, bwq, bwo))

    def start_heads(br, h, slot, u, n):
        for kv in range(2):
            pltpu.make_async_copy(srcs[br][1 + kv].at[:, pl.ds(h, n)],
                                  kvb.at[slot, kv, :, pl.ds(u, n)], kvsem.at[slot]).start(priority=1)
        for c in range(NC):
            pltpu.make_async_copy(
                srcs[br][4].at[pl.ds(pl.multiple_of(h * DH, DH), n * DH), pl.ds(c * 128, 128)],
                wob.at[slot, c, pl.ds(pl.multiple_of(u * DH, DH), n * DH)], wosem.at[slot]).start(priority=1)

    def wait_slot(slot):
        pltpu.make_async_copy(kvb.at[slot], kvb.at[slot], kvsem.at[slot]).wait()
        pltpu.make_async_copy(wob.at[slot], wob.at[slot], wosem.at[slot]).wait()

    def start_wq(br, g, slot, sem, u0=0, u1=GQ):
        for u in range(u0, u1):
            h = g * GQ + u
            pltpu.make_async_copy(srcs[br][3].at[:, pl.ds(pl.multiple_of(h * DH, DH), DH)],
                                  wqb.at[slot, u], sem).start()

    def wait_wq(slot, sem, u0=0, u1=GQ):
        pltpu.make_async_copy(wqb.at[slot, u0:u1], wqb.at[slot, u0:u1], sem).wait()

    def start_x(br, sem, r0=0, r1=M):
        for c in range(NC):
            pltpu.make_async_copy(srcs[br][0].at[r0:r1, pl.ds(c * 128, 128)], xs.at[br, c, r0:r1], sem).start()

    def wait_x(br, sem, r0=0, r1=M):
        pltpu.make_async_copy(xs.at[br, :, r0:r1], xs.at[br, :, r0:r1], sem).wait()

    def out_copies(br, b):
        rows = pl.ds(b * SQ, SQ)
        return [pltpu.make_async_copy(stage.at[br, c, rows],
                                      out.at[rows, pl.ds(pl.multiple_of(br * D + c * 128, 128), 128)],
                                      osem.at[br]) for c in range(NC)]

    def q_unit(br, slot, t0, b, u):
        rows = pl.ds(b * SQ, SQ)
        r = None
        for c in range(NC):
            d = _dot(_ld(xs.at[br, c, rows]), _ld(wqb.at[slot, u, pl.ds(c * 128, 128)]))
            r = d if r is None else r + d
        qall[t0 + u, rows, :] = (r * QSCALE).astype(jnp.bfloat16)

    def q_prefetch(j, pslot):
        g = j + NQ - 1

        @pl.when(g < NJB)
        def _():
            start_wq(0, g, pslot, qsem.at[pslot])

        @pl.when(jnp.logical_and(g >= NJB, g < NJ))
        def _():
            start_wq(1, g - NJB, pslot, qsem.at[pslot])

        t = (j + 1) * HPJ

        @pl.when(j + 1 < NJ)
        def _():
            start_heads(0, t, t // G, t % G, HPJ)

        @pl.when(j == 1)
        def _():
            start_x(1, psem.at[4])

    hb, hu = B // 2, GQ // 2
    start_x(0, psem.at[0], 0, hb * SQ)
    start_wq(0, 0, 0, psem.at[1], 0, hu)
    acc[...] = jnp.zeros_like(acc)
    wait_x(0, psem.at[0], 0, hb * SQ)
    start_x(0, psem.at[2], hb * SQ, M)
    start_wq(0, 0, 0, psem.at[3], hu, GQ)
    wait_wq(0, psem.at[1], 0, hu)
    for b in range(hb):
        for u in range(hu):
            q_unit(0, 0, 0, b, u)
            if b == 0 and u == 0:
                start_wq(0, 1, 1, qsem.at[1])
                start_heads(0, 0, 0, 0, HPJ)
    wait_x(0, psem.at[2], hb * SQ, M)
    wait_wq(0, psem.at[3], hu, GQ)
    first = True
    for b in range(B):
        for u in range(GQ):
            if b < hb and u < hu:
                continue
            q_unit(0, 0, 0, b, u)
            if first:
                first = False
                start_wq(0, 2, 2, qsem.at[2])
                start_heads(0, HPJ, HPJ // G, HPJ % G, HPJ)

    def q_body(j, carry):
        slot, pslot = carry
        br = j >> (NJB.bit_length() - 1)

        @pl.when(j == NJB)
        def _():
            wait_x(1, psem.at[4])

        wait_wq(slot, qsem.at[slot])
        for b in range(B):
            for u in range(GQ):
                q_unit(br, slot, j * GQ, b, u)
                if b == 0 and u == 3:
                    q_prefetch(j, pslot)
        return jnp.where(slot == NQ - 1, 0, slot + 1), slot

    lax.fori_loop(1, NJ, q_body, (jnp.int32(1), jnp.int32(0)))

    def attend(heads, toks, h0, br, slot0, last, prefetch):
        for s in range(heads // G):
            wait_slot(slot0 + s)

        def scores(n):
            u, b = divmod(n, B)
            q = _ld(qall.at[h0 + u, pl.ds(b * SQ, SQ)])
            k = _ld(kvb.at[slot0 + u // G, 0, b, u % G])
            s = lax.dot_general(q, k, (((1,), (1,)), ((), ())), preferred_element_type=jnp.float32)
            m = jnp.max(s, axis=-1, keepdims=True)
            p = jnp.exp2(s - m)
            l = jnp.sum(p, axis=-1, keepdims=True)
            r0 = pl.reciprocal(l, approx=True)
            return p.astype(jnp.bfloat16), r0 * (2.0 - l * r0)

        def pv(n, p, rl):
            u, b = divmod(n, B)
            return (_dot(p, _ld(kvb.at[slot0 + u // G, 1, b, u % G])) * rl).astype(jnp.bfloat16)

        def out_proj(n, o):
            u, b = divmod(n, B)
            rows = pl.ds(b * SQ, SQ)
            uu = u % G
            for c in range(NC):
                cols = slice(c * 128, (c + 1) * 128)
                new = acc[br, rows, cols] + _dot(o, _ld(wob.at[slot0 + u // G, c, uu * DH:(uu + 1) * DH]))
                acc[br, rows, cols] = new
                if u == heads - 1:
                    stage[br, c, rows, :] = new.astype(jnp.bfloat16)
            if u == heads - 1:
                @pl.when(last)
                def _():
                    for cp in out_copies(br, b):
                        cp.start()

        soft, o_val = {}, {}
        for kind, n in toks:
            if kind == "S":
                soft[n] = scores(n)
            elif kind == "P":
                o_val[n] = pv(n, *soft.pop(n))
            elif kind == "O":
                out_proj(n, o_val.pop(n))
            else:
                prefetch(n)

    toks8 = _order(8, (1, 33))
    toks4 = _order(4, ())

    def body8(i, slot0):
        pslot = jnp.where(slot0 == 0, NS - 2, slot0 - 2)

        def prefetch(k):
            it = i + 2
            h = it * 8 + k * G

            @pl.when(it < 4)
            def _():
                start_heads(0, h, pslot + k, 0, G)

            @pl.when(it >= 4)
            def _():
                start_heads(1, h - H, pslot + k, 0, G)

        attend(8, toks8, i * 8, i >> 2, slot0, i == 3, prefetch)
        return jnp.where(slot0 == NS - 2, 0, slot0 + 2)

    lax.fori_loop(0, N8, body8, jnp.int32(0))

    def body4(k, carry):
        attend(4, toks4, 8 * N8 + 4 * k, 1, (2 * N8) % NS + k, k == N4 - 1, None)
        return carry

    lax.fori_loop(0, N4, body4, None)

    for br in range(2):
        for b in range(B):
            for cp in out_copies(br, b):
                cp.wait()


@jax.jit
def pallas_concat_heads__mha_block_cached__mha_block_cached__near_ridge_kernel(
    A_x: jax.Array,
    A_k_cache: jax.Array,
    A_v_cache: jax.Array,
    A_wq: jax.Array,
    A_wo: jax.Array,
    B_x: jax.Array,
    B_k_cache: jax.Array,
    B_v_cache: jax.Array,
    B_wq: jax.Array,
    B_wo: jax.Array,
):
    hbm = pl.BlockSpec(memory_space=pl.ANY)
    out = pl.pallas_call(
        _kernel,
        in_specs=[hbm] * 10,
        out_specs=hbm,
        out_shape=jax.ShapeDtypeStruct((M, 2 * D), jnp.bfloat16),
        scratch_shapes=[
            pltpu.VMEM((2, NC, M, 128), jnp.bfloat16),
            pltpu.VMEM((NS, 2, B, G, SK, DH), jnp.bfloat16),
            pltpu.VMEM((NQ, GQ, D, DH), jnp.bfloat16),
            pltpu.VMEM((NS, NC, G * DH, 128), jnp.bfloat16),
            pltpu.VMEM((2 * H, M, DH), jnp.bfloat16),
            pltpu.VMEM((2, M, D), jnp.float32),
            pltpu.VMEM((2, NC, M, 128), jnp.bfloat16),
            pltpu.SemaphoreType.DMA((NS,)),
            pltpu.SemaphoreType.DMA((NS,)),
            pltpu.SemaphoreType.DMA((NQ,)),
            pltpu.SemaphoreType.DMA((5,)),
            pltpu.SemaphoreType.DMA((2,)),
        ],
        compiler_params=pltpu.CompilerParams(
            vmem_limit_bytes=110 * 1024 * 1024, disable_bounds_checks=True),
    )(A_x.reshape(M, D), A_k_cache, A_v_cache, A_wq, A_wo,
      B_x.reshape(M, D), B_k_cache, B_v_cache, B_wq, B_wo)
    return out.reshape(B, SQ, 2 * D)
```

```python
import math

import jax
import jax.numpy as jnp
from jax import lax
import jax.experimental.pallas as pl
import jax.experimental.pallas.tpu as pltpu

B, SQ, D = 8, 144, 640
H, SK, DH = 32, 512, 128
M = B * SQ
NC = D // 128
QSCALE = (DH ** -0.5) * math.log2(math.e)

GQ = 8
NJ = 2 * H // GQ
NJB = H // GQ
NQ = 3
G = 4
NS = 6
GA = 8
NI = 2 * H // GA
NIB = H // GA
HPJ = 2
STAGES = ((2, 2), (3, 3), (4, 4), (6, 6), (8, 8))
NST = len(STAGES)


def _order():
    n_units = GA * B
    toks = []
    for n in range(n_units + 2):
        if n < n_units:
            toks.append(("S", n))
        if 0 <= n - 1 < n_units:
            toks.append(("P", n - 1))
        if 0 <= n - 2 < n_units:
            toks.append(("O", n - 2))
        if n in (1, 33):
            toks.append(("D", n // 32))
    return toks


def _ld(ref):
    return pltpu.bitcast(ref.bitcast(jnp.uint32)[...], jnp.bfloat16)


def _dot(a, b):
    return jnp.dot(a, b, preferred_element_type=jnp.float32)


def _kernel(ax, ak, av, awq, awo, bx, bk, bv, bwq, bwo, out,
            xs, kvb, wqb, wob, qall, acc, stage, kvsem, wosem, qsem, psem, osem):
    srcs = ((ax, ak, av, awq, awo), (bx, bk, bv, bwq, bwo))

    def start_heads(br, h, slot, u, n, priority=1):
        for kv in range(2):
            pltpu.make_async_copy(srcs[br][1 + kv].at[:, pl.ds(h, n)],
                                  kvb.at[slot, kv, :, pl.ds(u, n)], kvsem.at[slot]).start(priority=priority)
        for c in range(NC):
            pltpu.make_async_copy(
                srcs[br][4].at[pl.ds(pl.multiple_of(h * DH, DH), n * DH), pl.ds(c * 128, 128)],
                wob.at[slot, c, pl.ds(pl.multiple_of(u * DH, DH), n * DH)],
                wosem.at[slot]).start(priority=priority)

    def wait_slot(slot):
        pltpu.make_async_copy(kvb.at[slot], kvb.at[slot], kvsem.at[slot]).wait()
        pltpu.make_async_copy(wob.at[slot], wob.at[slot], wosem.at[slot]).wait()

    def start_wq(br, g, slot, sem, u0=0, u1=GQ):
        for u in range(u0, u1):
            h = g * GQ + u
            pltpu.make_async_copy(srcs[br][3].at[:, pl.ds(pl.multiple_of(h * DH, DH), DH)],
                                  wqb.at[slot, u], sem).start()

    def wait_wq(slot, sem, u0=0, u1=GQ):
        pltpu.make_async_copy(wqb.at[slot, u0:u1], wqb.at[slot, u0:u1], sem).wait()

    def start_x(br, sem, r0=0, r1=M):
        for c in range(NC):
            pltpu.make_async_copy(srcs[br][0].at[r0:r1, pl.ds(c * 128, 128)], xs.at[br, c, r0:r1], sem).start()

    def wait_x(br, sem, r0=0, r1=M):
        pltpu.make_async_copy(xs.at[br, :, r0:r1], xs.at[br, :, r0:r1], sem).wait()

    def out_copies(br, b):
        rows = pl.ds(b * SQ, SQ)
        return [pltpu.make_async_copy(stage.at[br, c, rows],
                                      out.at[rows, pl.ds(pl.multiple_of(br * D + c * 128, 128), 128)],
                                      osem.at[br]) for c in range(NC)]

    def q_unit(br, slot, t0, b, u):
        rows = pl.ds(b * SQ, SQ)
        r = None
        for c in range(NC):
            d = _dot(_ld(xs.at[br, c, rows]), _ld(wqb.at[slot, u, pl.ds(c * 128, 128)]))
            r = d if r is None else r + d
        qall[t0 + u, rows, :] = (r * QSCALE).astype(jnp.bfloat16)

    lo = ((0, 0),) + STAGES[:-1]

    def issue(st, carry):
        for k in range(NST):
            @pl.when(st == k)
            def _():
                start_x(0, psem.at[2 * k], lo[k][0] * SQ, STAGES[k][0] * SQ)
                start_wq(0, 0, 0, psem.at[2 * k + 1], lo[k][1], STAGES[k][1])

        @pl.when(st == NST)
        def _():
            start_wq(0, 1, 1, qsem.at[1])

        @pl.when(st == NST + 1)
        def _():
            start_wq(0, 2, 2, qsem.at[2])

        @pl.when(st == NST + 2)
        def _():
            start_heads(0, 0, 0, 0, G, priority=0)
        return carry

    lax.fori_loop(0, NST + 3, issue, None)

    for k in range(NST):
        wait_x(0, psem.at[2 * k], lo[k][0] * SQ, STAGES[k][0] * SQ)
        wait_wq(0, psem.at[2 * k + 1], lo[k][1], STAGES[k][1])
        for b in range(STAGES[k][0]):
            for u in range(STAGES[k][1]):
                if b < lo[k][0] and u < lo[k][1]:
                    continue
                q_unit(0, 0, 0, b, u)

    def q_body(j, carry):
        slot, pslot = carry
        br = j >> (NJB.bit_length() - 1)

        @pl.when(j == NJB)
        def _():
            wait_x(1, psem.at[2 * NST])

        wait_wq(slot, qsem.at[slot])
        for b in range(B):
            for u in range(GQ):
                q_unit(br, slot, j * GQ, b, u)
                if b == 0 and u == 3:
                    g = j + NQ - 1

                    @pl.when(g < NJB)
                    def _():
                        start_wq(0, g, pslot, qsem.at[pslot])

                    @pl.when(jnp.logical_and(g >= NJB, g < NJ))
                    def _():
                        start_wq(1, g - NJB, pslot, qsem.at[pslot])

                    t = (j + 1) * HPJ

                    @pl.when(j + 1 < NJ)
                    def _():
                        start_heads(0, t, t >> 2, t & (G - 1), HPJ)

                    @pl.when(j == 1)
                    def _():
                        start_x(1, psem.at[2 * NST])
        return jnp.where(slot == NQ - 1, 0, slot + 1), slot

    lax.fori_loop(1, NJ, q_body, (jnp.int32(1), jnp.int32(0)))

    toks = _order()

    def attend(i, slot0):
        pslot = jnp.where(slot0 == 0, NS - 2, slot0 - 2)
        br = i >> (NIB.bit_length() - 1)
        first = (i & (NIB - 1)) == 0
        last = (i & (NIB - 1)) == NIB - 1
        wait_slot(slot0)

        def scores(n):
            u, b = divmod(n, B)
            q = _ld(qall.at[i * GA + u, pl.ds(b * SQ, SQ)])
            k = _ld(kvb.at[slot0 + u // G, 0, b, u % G])
            s = lax.dot_general(q, k, (((1,), (1,)), ((), ())), preferred_element_type=jnp.float32)
            m = jnp.max(s, axis=-1, keepdims=True)
            p = jnp.exp2(s - m)
            l = jnp.sum(p, axis=-1, keepdims=True)
            r0 = pl.reciprocal(l, approx=True)
            return p.astype(jnp.bfloat16), r0 * (2.0 - l * r0)

        def pv(n, p, rl):
            u, b = divmod(n, B)
            return (_dot(p, _ld(kvb.at[slot0 + u // G, 1, b, u % G])) * rl).astype(jnp.bfloat16)

        def out_proj(n, o):
            u, b = divmod(n, B)
            rows = pl.ds(b * SQ, SQ)
            uu = u % G
            for c in range(NC):
                cols = slice(c * 128, (c + 1) * 128)
                old = acc[br, rows, cols]
                if u == 0:
                    old = jnp.where(first, 0.0, old)
                new = old + _dot(o, _ld(wob.at[slot0 + u // G, c, uu * DH:(uu + 1) * DH]))
                acc[br, rows, cols] = new
                if u == GA - 1:
                    stage[br, c, rows, :] = new.astype(jnp.bfloat16)
            if u == GA - 1:
                @pl.when(last)
                def _():
                    for cp in out_copies(br, b):
                        cp.start()

        def prefetch(k):
            it = i + 2
            h = it * GA + k * G

            @pl.when(it < NIB)
            def _():
                start_heads(0, h, pslot + k, 0, G)

            @pl.when(jnp.logical_and(it >= NIB, it < NI))
            def _():
                start_heads(1, h - H, pslot + k, 0, G)

        soft, o_val = {}, {}
        for kind, n in toks:
            if kind == "S":
                if n == G * B:
                    wait_slot(slot0 + 1)
                soft[n] = scores(n)
            elif kind == "P":
                o_val[n] = pv(n, *soft.pop(n))
            elif kind == "O":
                out_proj(n, o_val.pop(n))
            else:
                prefetch(n)
        return jnp.where(slot0 == NS - 2, 0, slot0 + 2)

    lax.fori_loop(0, NI, attend, jnp.int32(0))

    for br in range(2):
        for b in range(B):
            for cp in out_copies(br, b):
                cp.wait()


@jax.jit
def pallas_concat_heads__mha_block_cached__mha_block_cached__near_ridge_kernel(
    A_x: jax.Array,
    A_k_cache: jax.Array,
    A_v_cache: jax.Array,
    A_wq: jax.Array,
    A_wo: jax.Array,
    B_x: jax.Array,
    B_k_cache: jax.Array,
    B_v_cache: jax.Array,
    B_wq: jax.Array,
    B_wo: jax.Array,
):
    hbm = pl.BlockSpec(memory_space=pl.ANY)
    out = pl.pallas_call(
        _kernel,
        in_specs=[hbm] * 10,
        out_specs=hbm,
        out_shape=jax.ShapeDtypeStruct((M, 2 * D), jnp.bfloat16),
        scratch_shapes=[
            pltpu.VMEM((2, NC, M, 128), jnp.bfloat16),
            pltpu.VMEM((NS, 2, B, G, SK, DH), jnp.bfloat16),
            pltpu.VMEM((NQ, GQ, D, DH), jnp.bfloat16),
            pltpu.VMEM((NS, NC, G * DH, 128), jnp.bfloat16),
            pltpu.VMEM((2 * H, M, DH), jnp.bfloat16),
            pltpu.VMEM((2, M, D), jnp.float32),
            pltpu.VMEM((2, NC, M, 128), jnp.bfloat16),
            pltpu.SemaphoreType.DMA((NS,)),
            pltpu.SemaphoreType.DMA((NS,)),
            pltpu.SemaphoreType.DMA((NQ,)),
            pltpu.SemaphoreType.DMA((2 * NST + 1,)),
            pltpu.SemaphoreType.DMA((2,)),
        ],
        compiler_params=pltpu.CompilerParams(
            vmem_limit_bytes=110 * 1024 * 1024,
            disable_bounds_checks=True,
            flags={"XLA_TPU_RESCHEDULE_DMA_DONES": True}),
    )(A_x.reshape(M, D), A_k_cache, A_v_cache, A_wq, A_wo,
      B_x.reshape(M, D), B_k_cache, B_v_cache, B_wq, B_wo)
    return out.reshape(B, SQ, 2 * D)
```

```python
import math

import jax
import jax.numpy as jnp
from jax import lax
import jax.experimental.pallas as pl
import jax.experimental.pallas.tpu as pltpu

B, SQ, D = 8, 144, 640
H, SK, DH = 32, 512, 128
M = B * SQ
NC = D // 128
QSCALE = (DH ** -0.5) * math.log2(math.e)

GQ = 8
NJ = 2 * H // GQ
NJB = H // GQ
NQ = 3
G = 4
NS = 6
GA = 8
NI = 2 * H // GA
NIB = H // GA
HPJ = 2
STAGES = ((2, 2), (3, 3), (4, 4), (6, 6), (8, 8))
NST = len(STAGES)


def _order():
    n_units = GA * B
    toks = []
    for n in range(n_units + 2):
        if n < n_units:
            toks.append(("S", n))
        if 0 <= n - 1 < n_units:
            toks.append(("P", n - 1))
        if 0 <= n - 2 < n_units:
            toks.append(("O", n - 2))
        if n in (1, 33):
            toks.append(("D", n // 32))
    return toks


def _dot(a, b):
    return jnp.dot(a, b, preferred_element_type=jnp.float32)


def _kernel(ax, ak, av, awq, awo, bx, bk, bv, bwq, bwo, out,
            xs, kvb, wqb, wob, qall, acc, stage, kvsem, wosem, qsem, psem, osem):
    srcs = ((ax, ak, av, awq, awo), (bx, bk, bv, bwq, bwo))

    def start_heads(br, h, slot, u, n, priority=1):
        for kv in range(2):
            pltpu.make_async_copy(srcs[br][1 + kv].at[:, pl.ds(h, n)],
                                  kvb.at[slot, kv, :, pl.ds(u, n)], kvsem.at[slot]).start(priority=priority)
        for c in range(NC):
            pltpu.make_async_copy(
                srcs[br][4].at[pl.ds(pl.multiple_of(h * DH, DH), n * DH), pl.ds(c * 128, 128)],
                wob.at[slot, c, pl.ds(pl.multiple_of(u * DH, DH), n * DH)],
                wosem.at[slot]).start(priority=priority)

    def wait_slot(slot):
        pltpu.make_async_copy(kvb.at[slot], kvb.at[slot], kvsem.at[slot]).wait()
        pltpu.make_async_copy(wob.at[slot], wob.at[slot], wosem.at[slot]).wait()

    def start_wq(br, g, slot, sem, u0=0, u1=GQ):
        for u in range(u0, u1):
            h = g * GQ + u
            pltpu.make_async_copy(srcs[br][3].at[:, pl.ds(pl.multiple_of(h * DH, DH), DH)],
                                  wqb.at[slot, u], sem).start()

    def wait_wq(slot, sem, u0=0, u1=GQ):
        pltpu.make_async_copy(wqb.at[slot, u0:u1], wqb.at[slot, u0:u1], sem).wait()

    def start_x(br, sem, r0=0, r1=M):
        for c in range(NC):
            pltpu.make_async_copy(srcs[br][0].at[r0:r1, pl.ds(c * 128, 128)], xs.at[br, c, r0:r1], sem).start()

    def wait_x(br, sem, r0=0, r1=M):
        pltpu.make_async_copy(xs.at[br, :, r0:r1], xs.at[br, :, r0:r1], sem).wait()

    def out_copies(br, b):
        rows = pl.ds(b * SQ, SQ)
        return [pltpu.make_async_copy(stage.at[br, c, rows],
                                      out.at[rows, pl.ds(pl.multiple_of(br * D + c * 128, 128), 128)],
                                      osem.at[br]) for c in range(NC)]

    def q_unit(br, slot, t0, b, u):
        rows = pl.ds(b * SQ, SQ)
        r = None
        for c in range(NC):
            d = _dot(xs[br, c, rows, :], wqb[slot, u, c * 128:(c + 1) * 128, :])
            r = d if r is None else r + d
        qall[t0 + u, rows, :] = (r * QSCALE).astype(jnp.bfloat16)

    lo = ((0, 0),) + STAGES[:-1]

    def issue(st, carry):
        for k in range(NST):
            @pl.when(st == k)
            def _():
                start_x(0, psem.at[2 * k], lo[k][0] * SQ, STAGES[k][0] * SQ)
                start_wq(0, 0, 0, psem.at[2 * k + 1], lo[k][1], STAGES[k][1])

        @pl.when(st == NST)
        def _():
            start_wq(0, 1, 1, qsem.at[1])

        @pl.when(st == NST + 1)
        def _():
            start_wq(0, 2, 2, qsem.at[2])

        @pl.when(st == NST + 2)
        def _():
            start_heads(0, 0, 0, 0, G, priority=0)
        return carry

    lax.fori_loop(0, NST + 3, issue, None)

    for k in range(NST):
        wait_x(0, psem.at[2 * k], lo[k][0] * SQ, STAGES[k][0] * SQ)
        wait_wq(0, psem.at[2 * k + 1], lo[k][1], STAGES[k][1])
        for b in range(STAGES[k][0]):
            for u in range(STAGES[k][1]):
                if b < lo[k][0] and u < lo[k][1]:
                    continue
                q_unit(0, 0, 0, b, u)

    def q_body(j, carry):
        slot, pslot = carry
        br = j >> (NJB.bit_length() - 1)

        @pl.when(j == NJB)
        def _():
            wait_x(1, psem.at[2 * NST])

        wait_wq(slot, qsem.at[slot])
        for b in range(B):
            for u in range(GQ):
                q_unit(br, slot, j * GQ, b, u)
                if b == 0 and u == 3:
                    g = j + NQ - 1

                    @pl.when(g < NJB)
                    def _():
                        start_wq(0, g, pslot, qsem.at[pslot])

                    @pl.when(jnp.logical_and(g >= NJB, g < NJ))
                    def _():
                        start_wq(1, g - NJB, pslot, qsem.at[pslot])

                    t = (j + 1) * HPJ

                    @pl.when(j + 1 < NJ)
                    def _():
                        start_heads(0, t, t >> 2, t & (G - 1), HPJ)

                    @pl.when(j == 1)
                    def _():
                        start_x(1, psem.at[2 * NST])
        return jnp.where(slot == NQ - 1, 0, slot + 1), slot

    lax.fori_loop(1, NJ, q_body, (jnp.int32(1), jnp.int32(0)))

    toks = _order()

    def attend(i, slot0):
        pslot = jnp.where(slot0 == 0, NS - 2, slot0 - 2)
        br = i >> (NIB.bit_length() - 1)
        first = (i & (NIB - 1)) == 0
        last = (i & (NIB - 1)) == NIB - 1
        wait_slot(slot0)

        def scores(n):
            u, b = divmod(n, B)
            q = qall[i * GA + u, pl.ds(b * SQ, SQ), :]
            k = kvb[slot0 + u // G, 0, b, u % G]
            s = lax.dot_general(q, k, (((1,), (1,)), ((), ())), preferred_element_type=jnp.float32)
            m = jnp.max(s, axis=-1, keepdims=True)
            p = jnp.exp2(s - m)
            l = jnp.sum(p, axis=-1, keepdims=True)
            r0 = pl.reciprocal(l, approx=True)
            return p.astype(jnp.bfloat16), r0 * (2.0 - l * r0)

        def pv(n, p, rl):
            u, b = divmod(n, B)
            return (_dot(p, kvb[slot0 + u // G, 1, b, u % G]) * rl).astype(jnp.bfloat16)

        def out_proj(n, o):
            u, b = divmod(n, B)
            rows = pl.ds(b * SQ, SQ)
            uu = u % G
            for c in range(NC):
                cols = slice(c * 128, (c + 1) * 128)
                old = acc[br, rows, cols]
                if u == 0:
                    old = jnp.where(first, 0.0, old)
                new = old + _dot(o, wob[slot0 + u // G, c, uu * DH:(uu + 1) * DH, :])
                acc[br, rows, cols] = new
                if u == GA - 1:
                    stage[br, c, rows, :] = new.astype(jnp.bfloat16)
            if u == GA - 1:
                @pl.when(last)
                def _():
                    for cp in out_copies(br, b):
                        cp.start()

        def prefetch(k):
            it = i + 2
            h = it * GA + k * G

            @pl.when(it < NIB)
            def _():
                start_heads(0, h, pslot + k, 0, G)

            @pl.when(jnp.logical_and(it >= NIB, it < NI))
            def _():
                start_heads(1, h - H, pslot + k, 0, G)

        soft, o_val = {}, {}
        for kind, n in toks:
            if kind == "S":
                if n == G * B:
                    wait_slot(slot0 + 1)
                soft[n] = scores(n)
            elif kind == "P":
                o_val[n] = pv(n, *soft.pop(n))
            elif kind == "O":
                out_proj(n, o_val.pop(n))
            else:
                prefetch(n)
        return jnp.where(slot0 == NS - 2, 0, slot0 + 2)

    lax.fori_loop(0, NI, attend, jnp.int32(0))

    for br in range(2):
        for b in range(B):
            for cp in out_copies(br, b):
                cp.wait()


@jax.jit
def pallas_concat_heads__mha_block_cached__mha_block_cached__near_ridge_kernel(
    A_x: jax.Array,
    A_k_cache: jax.Array,
    A_v_cache: jax.Array,
    A_wq: jax.Array,
    A_wo: jax.Array,
    B_x: jax.Array,
    B_k_cache: jax.Array,
    B_v_cache: jax.Array,
    B_wq: jax.Array,
    B_wo: jax.Array,
):
    hbm = pl.BlockSpec(memory_space=pl.ANY)
    out = pl.pallas_call(
        _kernel,
        in_specs=[hbm] * 10,
        out_specs=hbm,
        out_shape=jax.ShapeDtypeStruct((M, 2 * D), jnp.bfloat16),
        scratch_shapes=[
            pltpu.VMEM((2, NC, M, 128), jnp.bfloat16),
            pltpu.VMEM((NS, 2, B, G, SK, DH), jnp.bfloat16),
            pltpu.VMEM((NQ, GQ, D, DH), jnp.bfloat16),
            pltpu.VMEM((NS, NC, G * DH, 128), jnp.bfloat16),
            pltpu.VMEM((2 * H, M, DH), jnp.bfloat16),
            pltpu.VMEM((2, M, D), jnp.float32),
            pltpu.VMEM((2, NC, M, 128), jnp.bfloat16),
            pltpu.SemaphoreType.DMA((NS,)),
            pltpu.SemaphoreType.DMA((NS,)),
            pltpu.SemaphoreType.DMA((NQ,)),
            pltpu.SemaphoreType.DMA((2 * NST + 1,)),
            pltpu.SemaphoreType.DMA((2,)),
        ],
        compiler_params=pltpu.CompilerParams(
            vmem_limit_bytes=110 * 1024 * 1024,
            disable_bounds_checks=True,
            disable_semaphore_checks=True,
            flags={"XLA_TPU_RESCHEDULE_DMA_DONES": True}),
    )(A_x.reshape(M, D), A_k_cache, A_v_cache, A_wq, A_wo,
      B_x.reshape(M, D), B_k_cache, B_v_cache, B_wq, B_wo)
    return out.reshape(B, SQ, 2 * D)
```

```python
import math

import jax
import jax.numpy as jnp
from jax import lax
import jax.experimental.pallas as pl
import jax.experimental.pallas.tpu as pltpu

B, SQ, D = 8, 144, 640
H, SK, DH = 32, 512, 128
M = B * SQ
NC = D // 128
QSCALE = (DH ** -0.5) * math.log2(math.e)

GQ = 8
NJ = 2 * H // GQ
NJB = H // GQ
NQ = 3
G = 4
NS = 6
GA = 8
NI = 2 * H // GA
NIB = H // GA
HPJ = 2
STAGES = ((1, 1), (2, 2), (3, 3), (4, 4), (5, 5), (8, 8))
NST = len(STAGES)


def _order():
    n_units = GA * B
    toks = []
    for n in range(n_units + 2):
        if n < n_units:
            toks.append(("S", n))
        if 0 <= n - 1 < n_units:
            toks.append(("P", n - 1))
        if 0 <= n - 2 < n_units:
            toks.append(("O", n - 2))
        if n in (1, 33):
            toks.append(("D", n // 32))
    return toks


def _dot(a, b):
    return jnp.dot(a, b, preferred_element_type=jnp.float32)


def _kernel(ax, ak, av, awq, awo, bx, bk, bv, bwq, bwo, out,
            xs, kvb, wqb, wob, qall, acc, stage, kvsem, wosem, qsem, psem, osem):
    srcs = ((ax, ak, av, awq, awo), (bx, bk, bv, bwq, bwo))

    def start_heads(br, h, slot, u, n, priority=1):
        for kv in range(2):
            pltpu.make_async_copy(srcs[br][1 + kv].at[:, pl.ds(h, n)],
                                  kvb.at[slot, kv, :, pl.ds(u, n)], kvsem.at[slot]).start(priority=priority)
        for c in range(NC):
            pltpu.make_async_copy(
                srcs[br][4].at[pl.ds(pl.multiple_of(h * DH, DH), n * DH), pl.ds(c * 128, 128)],
                wob.at[slot, c, pl.ds(pl.multiple_of(u * DH, DH), n * DH)],
                wosem.at[slot]).start(priority=priority)

    def wait_slot(slot):
        pltpu.make_async_copy(kvb.at[slot], kvb.at[slot], kvsem.at[slot]).wait()
        pltpu.make_async_copy(wob.at[slot], wob.at[slot], wosem.at[slot]).wait()

    def start_wq(br, g, slot, sem, u0=0, u1=GQ):
        for u in range(u0, u1):
            h = g * GQ + u
            pltpu.make_async_copy(srcs[br][3].at[:, pl.ds(pl.multiple_of(h * DH, DH), DH)],
                                  wqb.at[slot, u], sem).start()

    def wait_wq(slot, sem, u0=0, u1=GQ):
        pltpu.make_async_copy(wqb.at[slot, u0:u1], wqb.at[slot, u0:u1], sem).wait()

    def start_x(br, sem, r0=0, r1=M):
        for c in range(NC):
            pltpu.make_async_copy(srcs[br][0].at[r0:r1, pl.ds(c * 128, 128)], xs.at[br, c, r0:r1], sem).start()

    def wait_x(br, sem, r0=0, r1=M):
        pltpu.make_async_copy(xs.at[br, :, r0:r1], xs.at[br, :, r0:r1], sem).wait()

    def out_copies(br, b):
        rows = pl.ds(b * SQ, SQ)
        return [pltpu.make_async_copy(stage.at[br, c, rows],
                                      out.at[rows, pl.ds(pl.multiple_of(br * D + c * 128, 128), 128)],
                                      osem.at[br]) for c in range(NC)]

    def q_unit(br, slot, t0, b, u):
        rows = pl.ds(b * SQ, SQ)
        r = None
        for c in range(NC):
            d = _dot(xs[br, c, rows, :], wqb[slot, u, c * 128:(c + 1) * 128, :])
            r = d if r is None else r + d
        qall[t0 + u, rows, :] = (r * QSCALE).astype(jnp.bfloat16)

    lo = ((0, 0),) + STAGES[:-1]

    def issue(st, carry):
        for k in range(NST):
            @pl.when(st == k)
            def _():
                start_x(0, psem.at[2 * k], lo[k][0] * SQ, STAGES[k][0] * SQ)
                start_wq(0, 0, 0, psem.at[2 * k + 1], lo[k][1], STAGES[k][1])

        @pl.when(st == NST)
        def _():
            start_wq(0, 1, 1, qsem.at[1])

        @pl.when(st == NST + 1)
        def _():
            start_wq(0, 2, 2, qsem.at[2])

        @pl.when(st == NST + 2)
        def _():
            start_heads(0, 0, 0, 0, G, priority=0)
        return carry

    lax.fori_loop(0, NST + 3, issue, None)

    for k in range(NST):
        wait_x(0, psem.at[2 * k], lo[k][0] * SQ, STAGES[k][0] * SQ)
        wait_wq(0, psem.at[2 * k + 1], lo[k][1], STAGES[k][1])
        for b in range(lo[k][0], STAGES[k][0]):
            for u in range(lo[k][1]):
                q_unit(0, 0, 0, b, u)
        for u in range(lo[k][1], STAGES[k][1]):
            for b in range(STAGES[k][0]):
                q_unit(0, 0, 0, b, u)

    def q_body(j, carry):
        slot, pslot = carry
        br = j >> (NJB.bit_length() - 1)

        @pl.when(j == NJB)
        def _():
            wait_x(1, psem.at[2 * NST])

        wait_wq(slot, qsem.at[slot])
        for b in range(B):
            for u in range(GQ):
                q_unit(br, slot, j * GQ, b, u)
                if b == 0 and u == 3:
                    g = j + NQ - 1

                    @pl.when(g < NJB)
                    def _():
                        start_wq(0, g, pslot, qsem.at[pslot])

                    @pl.when(jnp.logical_and(g >= NJB, g < NJ))
                    def _():
                        start_wq(1, g - NJB, pslot, qsem.at[pslot])

                    t = (j + 1) * HPJ

                    @pl.when(j + 1 < NJ)
                    def _():
                        start_heads(0, t, t >> 2, t & (G - 1), HPJ)

                    @pl.when(j == 1)
                    def _():
                        start_x(1, psem.at[2 * NST])
        return jnp.where(slot == NQ - 1, 0, slot + 1), slot

    lax.fori_loop(1, NJ, q_body, (jnp.int32(1), jnp.int32(0)))

    toks = _order()

    def attend(i, slot0):
        pslot = jnp.where(slot0 == 0, NS - 2, slot0 - 2)
        br = i >> (NIB.bit_length() - 1)
        first = (i & (NIB - 1)) == 0
        last = (i & (NIB - 1)) == NIB - 1
        wait_slot(slot0)

        def scores(n):
            u, b = divmod(n, B)
            q = qall[i * GA + u, pl.ds(b * SQ, SQ), :]
            k = kvb[slot0 + u // G, 0, b, u % G]
            s = lax.dot_general(q, k, (((1,), (1,)), ((), ())), preferred_element_type=jnp.float32)
            m = jnp.max(s, axis=-1, keepdims=True)
            p = jnp.exp2(s - m)
            l = jnp.sum(p, axis=-1, keepdims=True)
            r0 = pl.reciprocal(l, approx=True)
            return p.astype(jnp.bfloat16), r0 * (2.0 - l * r0)

        def pv(n, p, rl):
            u, b = divmod(n, B)
            return (_dot(p, kvb[slot0 + u // G, 1, b, u % G]) * rl).astype(jnp.bfloat16)

        def out_proj(n, o):
            u, b = divmod(n, B)
            rows = pl.ds(b * SQ, SQ)
            uu = u % G
            for c in range(NC):
                cols = slice(c * 128, (c + 1) * 128)
                old = acc[br, rows, cols]
                if u == 0:
                    old = jnp.where(first, 0.0, old)
                new = old + _dot(o, wob[slot0 + u // G, c, uu * DH:(uu + 1) * DH, :])
                acc[br, rows, cols] = new
                if u == GA - 1:
                    stage[br, c, rows, :] = new.astype(jnp.bfloat16)
            if u == GA - 1:
                @pl.when(last)
                def _():
                    for cp in out_copies(br, b):
                        cp.start()

        def prefetch(k):
            it = i + 2
            h = it * GA + k * G

            @pl.when(it < NIB)
            def _():
                start_heads(0, h, pslot + k, 0, G)

            @pl.when(jnp.logical_and(it >= NIB, it < NI))
            def _():
                start_heads(1, h - H, pslot + k, 0, G)

        soft, o_val = {}, {}
        for kind, n in toks:
            if kind == "S":
                if n == G * B:
                    wait_slot(slot0 + 1)
                soft[n] = scores(n)
            elif kind == "P":
                o_val[n] = pv(n, *soft.pop(n))
            elif kind == "O":
                out_proj(n, o_val.pop(n))
            else:
                prefetch(n)
        return jnp.where(slot0 == NS - 2, 0, slot0 + 2)

    lax.fori_loop(0, NI, attend, jnp.int32(0))

    for br in range(2):
        for b in range(B):
            for cp in out_copies(br, b):
                cp.wait()


@jax.jit
def pallas_concat_heads__mha_block_cached__mha_block_cached__near_ridge_kernel(
    A_x: jax.Array,
    A_k_cache: jax.Array,
    A_v_cache: jax.Array,
    A_wq: jax.Array,
    A_wo: jax.Array,
    B_x: jax.Array,
    B_k_cache: jax.Array,
    B_v_cache: jax.Array,
    B_wq: jax.Array,
    B_wo: jax.Array,
):
    hbm = pl.BlockSpec(memory_space=pl.ANY)
    out = pl.pallas_call(
        _kernel,
        in_specs=[hbm] * 10,
        out_specs=hbm,
        out_shape=jax.ShapeDtypeStruct((M, 2 * D), jnp.bfloat16),
        scratch_shapes=[
            pltpu.VMEM((2, NC, M, 128), jnp.bfloat16),
            pltpu.VMEM((NS, 2, B, G, SK, DH), jnp.bfloat16),
            pltpu.VMEM((NQ, GQ, D, DH), jnp.bfloat16),
            pltpu.VMEM((NS, NC, G * DH, 128), jnp.bfloat16),
            pltpu.VMEM((2 * H, M, DH), jnp.bfloat16),
            pltpu.VMEM((2, M, D), jnp.float32),
            pltpu.VMEM((2, NC, M, 128), jnp.bfloat16),
            pltpu.SemaphoreType.DMA((NS,)),
            pltpu.SemaphoreType.DMA((NS,)),
            pltpu.SemaphoreType.DMA((NQ,)),
            pltpu.SemaphoreType.DMA((2 * NST + 1,)),
            pltpu.SemaphoreType.DMA((2,)),
        ],
        compiler_params=pltpu.CompilerParams(
            vmem_limit_bytes=110 * 1024 * 1024,
            disable_bounds_checks=True,
            disable_semaphore_checks=True,
            flags={"XLA_TPU_RESCHEDULE_DMA_DONES": True}),
    )(A_x.reshape(M, D), A_k_cache, A_v_cache, A_wq, A_wo,
      B_x.reshape(M, D), B_k_cache, B_v_cache, B_wq, B_wo)
    return out.reshape(B, SQ, 2 * D)
```
